```python
import os as _os
_os.environ.setdefault("JAX_PLATFORMS", "cpu")
import jax
import jax.numpy as jnp

def _softmax(x, axis=-1):
    return jax.nn.softmax(x, axis=axis)
def _gelu(x):
    return jax.nn.gelu(x, approximate=True)
def _silu(x):
    return jax.nn.silu(x)
def _sigmoid(x):
    return jax.nn.sigmoid(x)
def _layernorm(x, axis=-1, eps=1e-5):
    m = jnp.mean(x, axis=axis, keepdims=True)
    v = jnp.var(x, axis=axis, keepdims=True)
    return (x - m) / jnp.sqrt(v + eps)
def _scatter_add(tgt, idx, src, axis=0):
    return tgt.at[idx].add(src)
def _segment_sum(src, seg, n):
    return jax.ops.segment_sum(src, seg, n)
class _Rng:
    def __init__(self, key):
        self._k = key
    def _next(self):
        self._k, sub = jax.random.split(self._k)
        return sub
    def normal(self, shape):
        return jax.random.normal(self._next(), shape, dtype=jnp.bfloat16)
    def randint(self, lo, hi, shape):
        return jax.random.randint(self._next(), shape, lo, hi, dtype=jnp.int32)
    def uniform(self, shape, lo=0.0, hi=1.0):
        return jax.random.uniform(self._next(), shape, jnp.bfloat16, lo, hi)
    def permutation(self, n):
        return jax.random.permutation(self._next(), n)


kernel_name = 'sequential_preLN__sliding_local_dilated__dense_activation_relu__prompt'

def setup_inputs():
    _rng = _Rng(jax.random.key(int.from_bytes(__import__("os").urandom(4), "little")))
    _w = (lambda a: (lambda t: t.astype(jnp.bfloat16) if jnp.issubdtype(t.dtype, jnp.floating) else t)(jnp.asarray(a)))
    def _A_setup():
        B, S, D = 1, 2048, 1024
        return {
            "x": _w((lambda *s: _rng.normal(s) * 0.05)(B, S, D)),
            "wqkv": _w((lambda *s: _rng.normal(s) * 0.05)(D, 3 * D)),
            "wo": _w((lambda *s: _rng.normal(s) * 0.05)(D, D)),
        }
    _A_in = _A_setup()

    def _B_setup():
        B, S, D, Dff = 1, 2048, 1024, 3584
        return {
            "x": _w((lambda *s: _rng.normal(s) * 0.05)(B, S, D)),
            "w1": _w((lambda *s: _rng.normal(s) * 0.05)(D, Dff)),
            "w2": _w((lambda *s: _rng.normal(s) * 0.05)(Dff, D)),
        }
    _B_in = _B_setup()

    return {
        "A_x": _A_in["x"],
        "A_wqkv": _A_in["wqkv"],
        "A_wo": _A_in["wo"],
        "B_x": _B_in["x"],
        "B_w1": _B_in["w1"],
        "B_w2": _B_in["w2"],
    }

def reference(A_x, A_wqkv, A_wo, B_x, B_w1, B_w2):
    def _A_ref(x, wqkv, wo):
        B, S, D = x.shape
        H = 32; Dh = D // H
        W, dil = 8, 2
        qkv = (lambda x, *d: x.transpose(*d))((x @ wqkv).reshape(B, S, 3, H, Dh), 2, 0, 3, 1, 4)
        q, k, v = qkv[0], qkv[1], qkv[2]
        scale = Dh ** -0.5
        pos = jnp.arange(S)
        off = jnp.arange(W) * dil
        idx = pos[:, None] - off[None, :]
        mask = idx >= 0
        idx_c = jnp.where(mask, idx, 0).reshape(-1)
        kg = k[:, :, idx_c, :].reshape(B, H, S, W, Dh)
        vg = v[:, :, idx_c, :].reshape(B, H, S, W, Dh)
        logits = jnp.einsum("bhsd,bhswd->bhsw", q, kg) * scale
        logits = jnp.where(mask[None, None, :, :], logits, -1e9)
        attn = _softmax(logits, axis=-1)
        o = jnp.einsum("bhsw,bhswd->bhsd", attn, vg)
        return (lambda x, *d: x.transpose(*d))(o, 0, 2, 1, 3).reshape(B, S, D) @ wo

    def _B_ref(x, w1, w2):
        h = jnp.einsum("bsd,df->bsf", x, w1)
        zero = jnp.zeros_like(h)
        h = jnp.maximum(h, zero)
        return jnp.einsum("bsf,fd->bsd", h, w2)

    x = A_x
    h = x + _A_ref(_layernorm(x, axis=-1), A_wqkv, A_wo)
    h2 = h + _B_ref(_layernorm(h, axis=-1), B_w1, B_w2)
    return h2
```

```python
import functools
import jax
import jax.numpy as jnp
from jax import lax
import jax.experimental.pallas as pl
import jax.experimental.pallas.tpu as pltpu

S, D, H, DH, W, DIL, DFF = 2048, 1024, 32, 32, 8, 2, 3584
NB = D // 128
HALO = (W - 1) * DIL
EPS = 1e-5
NEG = -1e9
F32 = jnp.float32
BF16 = jnp.bfloat16


def _ln(xf):
    m = jnp.mean(xf, axis=-1, keepdims=True)
    c = xf - m
    v = jnp.mean(c * c, axis=-1, keepdims=True)
    return c * lax.rsqrt(v + EPS)


def make_kernel(R, FC, AR, PC, AG):
    G = R // 8
    NBLK = S // R
    NFC = DFF // FC
    scale = float(DH) ** -0.5

    def kernel(x0_ref, xn_ref, wqkv_hbm, wo_hbm, w1_hbm, w2_hbm, o_ref,
               wqkv_r, wqkv_s, wo_raw, wo_f, wo_s, w1_s, w2_s,
               xf_s, xo_s, xp_s, h_s, acc_s, q_s, kext, vext, ob_s, ln1_s, ln2_s, sems, fsems):
        i = pl.program_id(0)

        cp_p = [pltpu.make_async_copy(wqkv_hbm.at[:, p * D:(p + 1) * D], wqkv_r.at[:, p * D:(p + 1) * D], sems.at[p])
                for p in range(3)]
        cp_wo = pltpu.make_async_copy(wo_hbm, wo_raw, sems.at[3])

        def cp_w1(f):
            f0 = f * FC if isinstance(f, int) else pl.multiple_of(f * FC, FC)
            return pltpu.make_async_copy(w1_hbm.at[:, pl.ds(f0, FC)], w1_s.at[:, pl.ds(f0, FC)], fsems.at[0, f])

        def cp_w2(f):
            f0 = f * FC if isinstance(f, int) else pl.multiple_of(f * FC, FC)
            return pltpu.make_async_copy(w2_hbm.at[pl.ds(f0, FC), :], w2_s.at[pl.ds(f0, FC), :], fsems.at[1, f])

        def stage_x(x_ref, slot):
            for c in range(NB):
                xf_s[c] = x_ref[:, c * 128:(c + 1) * 128].astype(F32)
            for g in range(G):
                for c in range(NB):
                    xp_s[slot, g * 8:(g + 1) * 8, c * 128:(c + 1) * 128] = xf_s[c, pl.ds(g, 8, stride=G), :]
            for r in range(R // AR):
                ln1_s[r * AR:(r + 1) * AR, :] = _ln(xp_s[slot, r * AR:(r + 1) * AR, :]).astype(BF16)

        def perm_w(p):
            lane = lax.broadcasted_iota(jnp.int32, (PC // 2, 128), 1)
            for r in range(D // PC):
                r0 = r * PC
                xs = [pltpu.bitcast(wqkv_r[r0:r0 + PC, p * D + b * 128: p * D + (b + 1) * 128], jnp.uint32)
                      for b in range(NB)]
                for kbit in range(3):
                    s = 4 << kbit
                    bit0 = (lane & s) == 0
                    new = list(xs)
                    for b in range(NB):
                        if b & (1 << kbit):
                            continue
                        b1 = b | (1 << kbit)
                        new[b] = jnp.where(bit0, xs[b], pltpu.roll(xs[b1], s, 1))
                        new[b1] = jnp.where(bit0, pltpu.roll(xs[b], 128 - s, 1), xs[b1])
                    xs = new
                for t in range(NB):
                    wqkv_s[r0:r0 + PC, p * D + t * 128: p * D + (t + 1) * 128] = pltpu.bitcast(xs[t], BF16)

        def prep_wo():
            for c in range(NB):
                wo_f[c] = wo_raw[:, c * 128:(c + 1) * 128].astype(F32)

            def body(t, carry):
                t0 = pl.multiple_of(t * 128, 128)
                for c in range(NB):
                    for hh in range(4):
                        for j in range(4):
                            rws = wo_f[c, pl.ds(hh * 32 + 4 * t + j, 8, stride=128), :]
                            xo_s[c, pl.ds(hh * 32 + j, 8, stride=4), :] = rws
                    wo_s[pl.ds(t0, 128), c * 128:(c + 1) * 128] = xo_s[c, 0:128, :].astype(BF16)
                return carry
            lax.fori_loop(0, NB, body, 0)

        def proj_q():
            q = jnp.dot(ln1_s[...], wqkv_s[:, 0:D], preferred_element_type=F32)
            q_s[...] = q * scale

        def proj_kv(p, ext):
            val = jnp.dot(ln1_s[...], wqkv_s[:, p * D:(p + 1) * D], preferred_element_type=F32)
            sub = lax.broadcasted_iota(jnp.int32, (HALO * 8, D), 0) % 8
            prev_tail = ext[G * 8:(G + HALO) * 8, :]
            cur_tail = val[(G - HALO) * 8:, :]
            a = pltpu.roll(cur_tail, 1, 0)
            b = pltpu.roll(prev_tail, HALO * 8 - 7, 0)
            ext[0:HALO * 8, :] = jnp.where(sub == 0, b, a)
            ext[HALO * 8:, :] = val

        def stage_att(masked):
            lane = lax.broadcasted_iota(jnp.int32, (AG, 128), 1)
            row = lax.broadcasted_iota(jnp.int32, (AG, 128), 0)
            for it in range(R // AG):
                r0 = it * AG
                qs = [q_s[r0:r0 + AG, c * 128:(c + 1) * 128] for c in range(NB)]
                rr = row + r0
                pos = i * R + (rr % 8) * G + rr // 8
                logits = []
                for w in range(W):
                    off = r0 + (HALO - DIL * w) * 8
                    p = None
                    for c in range(NB):
                        t = qs[c] * kext[off:off + AG, c * 128:(c + 1) * 128]
                        p = t if p is None else p + t
                    p = p + jnp.where(lane % 2 == 0, pltpu.roll(p, 127, 1), pltpu.roll(p, 1, 1))
                    p = p + jnp.where(lane % 4 < 2, pltpu.roll(p, 126, 1), pltpu.roll(p, 2, 1))
                    if masked and r0 // 8 < DIL * w:
                        p = jnp.where(pos >= DIL * w, p, NEG)
                    logits.append(p)
                m = logits[0]
                for w in range(1, W):
                    m = jnp.maximum(m, logits[w])
                es = [jnp.exp(l - m) for l in logits]
                den = es[0]
                for w in range(1, W):
                    den = den + es[w]
                inv = 1.0 / den
                for c in range(NB):
                    acc = None
                    for w in range(W):
                        off = r0 + (HALO - DIL * w) * 8
                        t = es[w] * vext[off:off + AG, c * 128:(c + 1) * 128]
                        acc = t if acc is None else acc + t
                    ob_s[r0:r0 + AG, c * 128:(c + 1) * 128] = (acc * inv).astype(BF16)

        def stage_wo(slot):
            att = jnp.dot(ob_s[...], wo_s[...], preferred_element_type=F32)
            h_s[slot] = xp_s[slot] + att

        def stage_ln2(slot):
            for r in range(R // AR):
                ln2_s[r * AR:(r + 1) * AR, :] = _ln(h_s[slot, r * AR:(r + 1) * AR, :]).astype(BF16)

        def stage_out(outp):
            for g in range(G):
                for c in range(NB):
                    xo_s[c, pl.ds(g, 8, stride=G), :] = outp[g * 8:(g + 1) * 8, c * 128:(c + 1) * 128]
            for c in range(NB):
                o_ref[:, c * 128:(c + 1) * 128] = xo_s[c].astype(BF16)

        def stage_ffn_out(slot):
            ln2 = ln2_s[...]
            acc = None
            for f in range(NFC):
                h1 = jnp.dot(ln2, w1_s[:, f * FC:(f + 1) * FC], preferred_element_type=F32)
                h1 = jnp.maximum(h1, 0.0).astype(BF16)
                t = jnp.dot(h1, w2_s[f * FC:(f + 1) * FC, :], preferred_element_type=F32)
                acc = t if acc is None else acc + t
            stage_out(h_s[slot] + acc)

        @pl.when(i == 0)
        def _():
            cp_p[0].start()
            cp_p[1].start()
            kext[...] = jnp.zeros_like(kext)
            vext[...] = jnp.zeros_like(vext)
            stage_x(x0_ref, 0)
            cp_p[0].wait()
            cp_p[2].start()
            perm_w(0)
            cp_p[1].wait()
            cp_wo.start()
            cp_w1(0).start()
            cp_w2(0).start()
            perm_w(1)
            cp_p[2].wait()
            for f in range(1, NFC):
                cp_w1(f).start()
                cp_w2(f).start()
            perm_w(2)
            cp_wo.wait()
            prep_wo()

        @pl.when(i <= 1)
        def _():
            slot = i % 2
            proj_q()
            proj_kv(1, kext)
            proj_kv(2, vext)
            stage_att(True)
            stage_x(xn_ref, 1 - slot)
            stage_wo(slot)

        @pl.when(jnp.logical_and(i > 1, i < NBLK))
        def _():
            slot = i % 2
            proj_q()
            proj_kv(1, kext)
            proj_kv(2, vext)
            stage_ln2(1 - slot)
            stage_ffn_out(1 - slot)
            stage_att(False)
            stage_x(xn_ref, 1 - slot)
            stage_wo(slot)

        @pl.when(jnp.logical_or(i == 1, i == NBLK))
        def _():
            slot = (i - 1) % 2
            stage_ln2(slot)
            acc_s[...] = h_s[slot]

            def body(f, carry):
                @pl.when(i == 1)
                def _():
                    cp_w1(f).wait()
                    cp_w2(f).wait()
                f0 = pl.multiple_of(f * FC, FC)
                h1 = jnp.dot(ln2_s[...], w1_s[:, pl.ds(f0, FC)], preferred_element_type=F32)
                h1 = jnp.maximum(h1, 0.0).astype(BF16)
                acc_s[...] += jnp.dot(h1, w2_s[pl.ds(f0, FC), :], preferred_element_type=F32)
                return carry
            lax.fori_loop(0, NFC, body, 0)
            stage_out(acc_s[...])

    scratch = [
        pltpu.VMEM((D, 3 * D), BF16),
        pltpu.VMEM((D, 3 * D), BF16),
        pltpu.VMEM((D, D), BF16),
        pltpu.VMEM((NB, D, 128), F32),
        pltpu.VMEM((D, D), BF16),
        pltpu.VMEM((D, DFF), BF16),
        pltpu.VMEM((DFF, D), BF16),
        pltpu.VMEM((NB, R, 128), F32),
        pltpu.VMEM((NB, R, 128), F32),
        pltpu.VMEM((2, R, D), F32),
        pltpu.VMEM((2, R, D), F32),
        pltpu.VMEM((R, D), F32),
        pltpu.VMEM((R, D), F32),
        pltpu.VMEM(((G + HALO) * 8, D), F32),
        pltpu.VMEM(((G + HALO) * 8, D), F32),
        pltpu.VMEM((R, D), BF16),
        pltpu.VMEM((R, D), BF16),
        pltpu.VMEM((R, D), BF16),
        pltpu.SemaphoreType.DMA((4,)),
        pltpu.SemaphoreType.DMA((2, NFC)),
    ]
    return kernel, scratch, NBLK


def run(A_x, A_wqkv, A_wo, B_x, B_w1, B_w2, R=128, FC=512, AR=32, PC=64, AG=16):
    kernel, scratch, NBLK = make_kernel(R, FC, AR, PC, AG)
    x = A_x.reshape(S, D)
    out = pl.pallas_call(
        kernel,
        grid=(NBLK + 1,),
        in_specs=[
            pl.BlockSpec((R, D), lambda i: (0, 0)),
            pl.BlockSpec((R, D), lambda i: (jnp.minimum(i + 1, NBLK - 1), 0)),
            pl.BlockSpec(memory_space=pl.ANY),
            pl.BlockSpec(memory_space=pl.ANY),
            pl.BlockSpec(memory_space=pl.ANY),
            pl.BlockSpec(memory_space=pl.ANY),
        ],
        out_specs=pl.BlockSpec((R, D), lambda i: (jnp.maximum(i - 1, 0), 0)),
        out_shape=jax.ShapeDtypeStruct((S, D), BF16),
        scratch_shapes=scratch,
        compiler_params=pltpu.CompilerParams(
            dimension_semantics=("arbitrary",),
            vmem_limit_bytes=110 * 1024 * 1024,
        ),
    )(x, x, A_wqkv, A_wo, B_w1, B_w2)
    return out.reshape(1, S, D)


@jax.jit
def pallas_sequential_preLN__sliding_local_dilated__dense_activation_relu__prompt_kernel(A_x, A_wqkv, A_wo, B_x, B_w1, B_w2):
    return run(A_x, A_wqkv, A_wo, B_x, B_w1, B_w2)
```

```python
import functools
import jax
import jax.numpy as jnp
from jax import lax
import jax.experimental.pallas as pl
import jax.experimental.pallas.tpu as pltpu

S, D, H, DH, W, DIL, DFF = 2048, 1024, 32, 32, 8, 2, 3584
NB = D // 128
HALO = (W - 1) * DIL
EPS = 1e-5
NEG = -1e9
F32 = jnp.float32
BF16 = jnp.bfloat16


def _ln(xf):
    m = jnp.mean(xf, axis=-1, keepdims=True)
    c = xf - m
    v = jnp.mean(c * c, axis=-1, keepdims=True)
    return c * lax.rsqrt(v + EPS)


def make_kernel(R, FC, AR, PC, AG, CH):
    G = R // 8
    NBLK = S // R
    NFC = DFF // FC
    scale = float(DH) ** -0.5

    def kernel(x0_ref, xn_ref, wqkv_hbm, wo_hbm, w1_hbm, w2_hbm, o_ref,
               wqkv_r, wqkv_s, wo_raw, wo_f, wo_s, w1_s, w2_s,
               xf_s, xo_s, xp_s, h_s, acc_s, q_s, kext, vext, ob_s, ln1_s, ln2_s, idx_s, sems, fsems):
        i = pl.program_id(0)

        @pl.when(i == 0)
        def _():
            idx_s[0] = R
        qpad = pl.multiple_of(idx_s[0], 8)

        cp_p = [pltpu.make_async_copy(wqkv_hbm.at[:, p * D:(p + 1) * D], wqkv_r.at[:, p * D:(p + 1) * D], sems.at[p])
                for p in range(3)]
        cp_wo = pltpu.make_async_copy(wo_hbm, wo_raw, sems.at[3])

        def cp_w1(f):
            f0 = f * FC if isinstance(f, int) else pl.multiple_of(f * FC, FC)
            return pltpu.make_async_copy(w1_hbm.at[:, pl.ds(f0, FC)], w1_s.at[:, pl.ds(f0, FC)], fsems.at[0, f])

        def cp_w2(f):
            f0 = f * FC if isinstance(f, int) else pl.multiple_of(f * FC, FC)
            return pltpu.make_async_copy(w2_hbm.at[pl.ds(f0, FC), :], w2_s.at[pl.ds(f0, FC), :], fsems.at[1, f])

        def stage_x(x_ref, slot):
            for c in range(NB):
                xf_s[c] = x_ref[:, c * 128:(c + 1) * 128].astype(F32)
            for g in range(G):
                for c in range(NB):
                    xp_s[slot, g * 8:(g + 1) * 8, c * 128:(c + 1) * 128] = xf_s[c, pl.ds(g, 8, stride=G), :]
            for r in range(R // AR):
                ln1_s[r * AR:(r + 1) * AR, :] = _ln(xp_s[slot, r * AR:(r + 1) * AR, :]).astype(BF16)

        def perm_w(p):
            lane = lax.broadcasted_iota(jnp.int32, (PC // 2, 128), 1)
            for r in range(D // PC):
                r0 = r * PC
                xs = [pltpu.bitcast(wqkv_r[r0:r0 + PC, p * D + b * 128: p * D + (b + 1) * 128], jnp.uint32)
                      for b in range(NB)]
                for kbit in range(3):
                    s = 4 << kbit
                    bit0 = (lane & s) == 0
                    new = list(xs)
                    for b in range(NB):
                        if b & (1 << kbit):
                            continue
                        b1 = b | (1 << kbit)
                        new[b] = jnp.where(bit0, xs[b], pltpu.roll(xs[b1], s, 1))
                        new[b1] = jnp.where(bit0, pltpu.roll(xs[b], 128 - s, 1), xs[b1])
                    xs = new
                for t in range(NB):
                    wqkv_s[r0:r0 + PC, p * D + t * 128: p * D + (t + 1) * 128] = pltpu.bitcast(xs[t], BF16)

        def prep_wo():
            for c in range(NB):
                wo_f[c] = wo_raw[:, c * 128:(c + 1) * 128].astype(F32)

            def body(t, carry):
                t0 = pl.multiple_of(t * 128, 128)
                for c in range(NB):
                    for hh in range(4):
                        for j in range(4):
                            rws = wo_f[c, pl.ds(hh * 32 + 4 * t + j, 8, stride=128), :]
                            xo_s[c, pl.ds(hh * 32 + j, 8, stride=4), :] = rws
                    wo_s[pl.ds(t0, 128), c * 128:(c + 1) * 128] = xo_s[c, 0:128, :].astype(BF16)
                return carry
            lax.fori_loop(0, NB, body, 0)

        def proj_q():
            q = jnp.dot(ln1_s[...], wqkv_s[:, 0:D], preferred_element_type=F32)
            q_s[0:R, :] = q * scale

        def proj_kv(p, ext):
            val = jnp.dot(ln1_s[...], wqkv_s[:, p * D:(p + 1) * D], preferred_element_type=F32)
            sub = lax.broadcasted_iota(jnp.int32, (HALO * 8, D), 0) % 8
            prev_tail = ext[G * 8:(G + HALO) * 8, :]
            cur_tail = val[(G - HALO) * 8:, :]
            a = pltpu.roll(cur_tail, 1, 0)
            b = pltpu.roll(prev_tail, HALO * 8 - 7, 0)
            ext[0:HALO * 8, :] = jnp.where(sub == 0, b, a)
            ext[HALO * 8:, :] = val

        def stage_att(masked, chain):
            lane = lax.broadcasted_iota(jnp.int32, (AG, 128), 1)
            row = lax.broadcasted_iota(jnp.int32, (AG, 128), 0)
            for it in range(R // AG):
                r0 = it * AG
                qs = [q_s[r0:r0 + AG, c * 128:(c + 1) * 128] for c in range(NB)]
                rr = row + r0
                pos = i * R + (rr % 8) * G + rr // 8
                logits = []
                for w in range(W):
                    off = r0 + (HALO - DIL * w) * 8
                    p = None
                    for c in range(NB):
                        t = qs[c] * kext[off:off + AG, c * 128:(c + 1) * 128]
                        p = t if p is None else p + t
                    p = p + jnp.where(lane % 2 == 0, pltpu.roll(p, 127, 1), pltpu.roll(p, 1, 1))
                    p = p + jnp.where(lane % 4 < 2, pltpu.roll(p, 126, 1), pltpu.roll(p, 2, 1))
                    if masked and r0 // 8 < DIL * w:
                        p = jnp.where(pos >= DIL * w, p, NEG)
                    logits.append(p)
                m = logits[0]
                for w in range(1, W):
                    m = jnp.maximum(m, logits[w])
                es = [jnp.exp(l - m) for l in logits]
                den = es[0]
                for w in range(1, W):
                    den = den + es[w]
                inv = 1.0 / den
                outs = []
                for c in range(NB):
                    acc = None
                    for w in range(W):
                        off = r0 + (HALO - DIL * w) * 8
                        t = es[w] * vext[off:off + AG, c * 128:(c + 1) * 128]
                        acc = t if acc is None else acc + t
                    outs.append(pltpu.bitcast((acc * inv).astype(BF16), jnp.uint32))
                lane2 = lax.broadcasted_iota(jnp.int32, (AG // 2, 128), 1)
                for kbit in range(3):
                    sh = 4 << kbit
                    bit0 = (lane2 & sh) == 0
                    new = list(outs)
                    for b in range(NB):
                        if b & (1 << kbit):
                            continue
                        b1 = b | (1 << kbit)
                        new[b] = jnp.where(bit0, outs[b], pltpu.roll(outs[b1], sh, 1))
                        new[b1] = jnp.where(bit0, pltpu.roll(outs[b], 128 - sh, 1), outs[b1])
                    outs = new
                for c in range(NB):
                    ob_s[r0:r0 + AG, c * 128:(c + 1) * 128] = pltpu.bitcast(outs[c], BF16)
                if chain:
                    q_s[pl.ds(qpad, 8), 0:128] = pltpu.bitcast(outs[NB - 1], F32)[0:8]

        def stage_wo(slot):
            att = jnp.dot(ob_s[...], wo_raw[...], preferred_element_type=F32)
            h_s[slot] = xp_s[slot] + att

        def stage_ln2(slot):
            for r in range(R // AR):
                ln2_s[r * AR:(r + 1) * AR, :] = _ln(h_s[slot, r * AR:(r + 1) * AR, :]).astype(BF16)

        def stage_out(outp):
            for g in range(G):
                for c in range(NB):
                    xo_s[c, pl.ds(g, 8, stride=G), :] = outp[g * 8:(g + 1) * 8, c * 128:(c + 1) * 128]
            for c in range(NB):
                o_ref[:, c * 128:(c + 1) * 128] = xo_s[c].astype(BF16)

        def stage_ffn_out(slot):
            ln2 = ln2_s[...]
            acc = None
            for f in range(NFC):
                h1 = jnp.dot(ln2, w1_s[:, f * FC:(f + 1) * FC], preferred_element_type=F32)
                h1 = jnp.maximum(h1, 0.0).astype(BF16)
                t = jnp.dot(h1, w2_s[f * FC:(f + 1) * FC, :], preferred_element_type=F32)
                acc = t if acc is None else acc + t
            stage_out(h_s[slot] + acc)

        @pl.when(i == 0)
        def _():
            cp_p[0].start()
            cp_p[1].start()
            kext[...] = jnp.zeros_like(kext)
            vext[...] = jnp.zeros_like(vext)
            stage_x(x0_ref, 0)
            cp_p[0].wait()
            cp_p[2].start()
            perm_w(0)
            cp_p[1].wait()
            cp_wo.start()
            cp_w1(0).start()
            cp_w2(0).start()
            perm_w(1)
            cp_p[2].wait()
            for f in range(1, NFC):
                cp_w1(f).start()
                cp_w2(f).start()
            perm_w(2)
            cp_wo.wait()

        @pl.when(i <= 1)
        def _():
            slot = i % 2
            proj_q()
            proj_kv(1, kext)
            proj_kv(2, vext)
            stage_att(True, False)
            stage_x(xn_ref, 1 - slot)
            stage_wo(slot)

        @pl.when(jnp.logical_and(i > 1, i < NBLK))
        def _():
            slot = i % 2
            proj_q()
            proj_kv(1, kext)
            proj_kv(2, vext)
            stage_ln2(1 - slot)
            stage_ffn_out(1 - slot)
            stage_att(False, True)
            stage_x(xn_ref, 1 - slot)
            stage_wo(slot)

        @pl.when(jnp.logical_or(i == 1, i == NBLK))
        def _():
            slot = (i - 1) % 2
            stage_ln2(slot)
            acc_s[...] = h_s[slot]

            def body(f, carry):
                @pl.when(i == 1)
                def _():
                    cp_w1(f).wait()
                    cp_w2(f).wait()
                f0 = pl.multiple_of(f * FC, FC)
                h1 = jnp.dot(ln2_s[...], w1_s[:, pl.ds(f0, FC)], preferred_element_type=F32)
                h1 = jnp.maximum(h1, 0.0).astype(BF16)
                acc_s[...] += jnp.dot(h1, w2_s[pl.ds(f0, FC), :], preferred_element_type=F32)
                return carry
            lax.fori_loop(0, NFC, body, 0)
            stage_out(acc_s[...])

    scratch = [
        pltpu.VMEM((D, 3 * D), BF16),
        pltpu.VMEM((D, 3 * D), BF16),
        pltpu.VMEM((D, D), BF16),
        pltpu.VMEM((NB, D, 128), F32),
        pltpu.VMEM((D, D), BF16),
        pltpu.VMEM((D, DFF), BF16),
        pltpu.VMEM((DFF, D), BF16),
        pltpu.VMEM((NB, R, 128), F32),
        pltpu.VMEM((NB, R, 128), F32),
        pltpu.VMEM((2, R, D), F32),
        pltpu.VMEM((2, R, D), F32),
        pltpu.VMEM((R, D), F32),
        pltpu.VMEM((R + 8, D), F32),
        pltpu.VMEM(((G + HALO) * 8, D), F32),
        pltpu.VMEM(((G + HALO) * 8, D), F32),
        pltpu.VMEM((R, D), BF16),
        pltpu.VMEM((R, D), BF16),
        pltpu.VMEM((R, D), BF16),
        pltpu.SMEM((1,), jnp.int32),
        pltpu.SemaphoreType.DMA((4,)),
        pltpu.SemaphoreType.DMA((2, NFC)),
    ]
    return kernel, scratch, NBLK


def run(A_x, A_wqkv, A_wo, B_x, B_w1, B_w2, R=128, FC=512, AR=32, PC=128, AG=16, CH=1):
    kernel, scratch, NBLK = make_kernel(R, FC, AR, PC, AG, CH)
    x = A_x.reshape(S, D)
    out = pl.pallas_call(
        kernel,
        grid=(NBLK + 1,),
        in_specs=[
            pl.BlockSpec((R, D), lambda i: (0, 0)),
            pl.BlockSpec((R, D), lambda i: (jnp.minimum(i + 1, NBLK - 1), 0)),
            pl.BlockSpec(memory_space=pl.ANY),
            pl.BlockSpec(memory_space=pl.ANY),
            pl.BlockSpec(memory_space=pl.ANY),
            pl.BlockSpec(memory_space=pl.ANY),
        ],
        out_specs=pl.BlockSpec((R, D), lambda i: (jnp.maximum(i - 1, 0), 0)),
        out_shape=jax.ShapeDtypeStruct((S, D), BF16),
        scratch_shapes=scratch,
        compiler_params=pltpu.CompilerParams(
            dimension_semantics=("arbitrary",),
            vmem_limit_bytes=110 * 1024 * 1024,
        ),
    )(x, x, A_wqkv, A_wo, B_w1, B_w2)
    return out.reshape(1, S, D)


@jax.jit
def pallas_sequential_preLN__sliding_local_dilated__dense_activation_relu__prompt_kernel(A_x, A_wqkv, A_wo, B_x, B_w1, B_w2):
    return run(A_x, A_wqkv, A_wo, B_x, B_w1, B_w2)
```

```python
import jax
import jax.numpy as jnp
from jax import lax
import jax.experimental.pallas as pl
import jax.experimental.pallas.tpu as pltpu

S, D, H, DH, W, DIL, DFF = 2048, 1024, 32, 32, 8, 2, 3584
NB = D // 128
HALO = (W - 1) * DIL
EPS = 1e-5
NEG = -1e9
F32 = jnp.float32
BF16 = jnp.bfloat16


def _ln(xf):
    m = jnp.mean(xf, axis=-1, keepdims=True)
    c = xf - m
    v = jnp.mean(c * c, axis=-1, keepdims=True)
    return c * lax.rsqrt(v + EPS)


def _butterfly(xs, rows):
    lane = lax.broadcasted_iota(jnp.int32, (rows, 128), 1)
    for kbit in range(3):
        s = 4 << kbit
        bit0 = (lane & s) == 0
        new = list(xs)
        for b in range(NB):
            if b & (1 << kbit):
                continue
            b1 = b | (1 << kbit)
            new[b] = jnp.where(bit0, xs[b], pltpu.roll(xs[b1], s, 1))
            new[b1] = jnp.where(bit0, pltpu.roll(xs[b], 128 - s, 1), xs[b1])
        xs = new
    return xs


def make_kernel(R, FC, AR, PC, AG, FC2):
    G = R // 8
    NBLK = S // R
    NFC = DFF // FC
    NF2 = DFF // FC2
    scale = float(DH) ** -0.5

    def kernel(x0_ref, xn_ref, wqkv_hbm, wo_hbm, w1_hbm, w2_hbm, o_ref,
               wqkv_r, wqkv_s, wo_s, w1_s, w2_s,
               xf_s, xo_s, xp_s, h_s, acc_s, q_s, kext, vext, ob_s, ln1_s, ln2_s,
               lnp_s, stg_s, idx_s, sems, fsems):
        i = pl.program_id(0)

        @pl.when(i == 0)
        def _():
            idx_s[0] = R
        qpad = pl.multiple_of(idx_s[0], 8)

        cp_p = [pltpu.make_async_copy(wqkv_hbm.at[:, p * D:(p + 1) * D],
                                      wqkv_r.at[:, p * D:(p + 1) * D], sems.at[p])
                for p in range(3)]
        cp_wo = pltpu.make_async_copy(wo_hbm, wo_s, sems.at[3])

        def cp_w1(f):
            f0 = f * FC2 if isinstance(f, int) else pl.multiple_of(f * FC2, 128)
            return pltpu.make_async_copy(w1_hbm.at[:, pl.ds(f0, FC2)],
                                         w1_s.at[:, pl.ds(f0, FC2)], fsems.at[0, f])

        def cp_w2(f):
            f0 = f * FC2 if isinstance(f, int) else pl.multiple_of(f * FC2, 128)
            return pltpu.make_async_copy(w2_hbm.at[pl.ds(f0, FC2), :],
                                         w2_s.at[pl.ds(f0, FC2), :], fsems.at[1, f])

        def stage_x(x_ref, slot, ln_dst):
            for c in range(NB):
                xf_s[c] = x_ref[:, c * 128:(c + 1) * 128].astype(F32)
            for g in range(G):
                for c in range(NB):
                    xp_s[slot, g * 8:(g + 1) * 8, c * 128:(c + 1) * 128] = xf_s[c, pl.ds(g, 8, stride=G), :]
            for r in range(R // AR):
                ln_dst[r * AR:(r + 1) * AR, :] = _ln(xp_s[slot, r * AR:(r + 1) * AR, :]).astype(BF16)

        def perm_w(p):
            for r in range(D // PC):
                r0 = r * PC
                xs = [pltpu.bitcast(wqkv_r[r0:r0 + PC, p * D + b * 128: p * D + (b + 1) * 128], jnp.uint32)
                      for b in range(NB)]
                xs = _butterfly(xs, PC // 2)
                for t in range(NB):
                    wqkv_s[r0:r0 + PC, p * D + t * 128: p * D + (t + 1) * 128] = pltpu.bitcast(xs[t], BF16)

        def put_q(q):
            q_s[0:R, :] = q * scale

        def put_kv(ext, val):
            sub = lax.broadcasted_iota(jnp.int32, (HALO * 8, D), 0) % 8
            prev_tail = ext[G * 8:(G + HALO) * 8, :]
            cur_tail = val[(G - HALO) * 8:, :]
            a = pltpu.roll(cur_tail, 1, 0)
            b = pltpu.roll(prev_tail, HALO * 8 - 7, 0)
            ext[0:HALO * 8, :] = jnp.where(sub == 0, b, a)
            ext[HALO * 8:, :] = val

        def proj(p):
            return jnp.dot(ln1_s[...], wqkv_s[:, p * D:(p + 1) * D], preferred_element_type=F32)

        def proj2(p):
            val = jnp.dot(lnp_s[...], wqkv_s[:, p * D:(p + 1) * D], preferred_element_type=F32)
            stg_s[:, p * D:(p + 1) * D] = val[R:2 * R, :]
            return val[0:R, :]

        def stage_att(masked, chain):
            lane = lax.broadcasted_iota(jnp.int32, (AG, 128), 1)
            row = lax.broadcasted_iota(jnp.int32, (AG, 128), 0)
            for it in range(R // AG):
                r0 = it * AG
                qs = [q_s[r0:r0 + AG, c * 128:(c + 1) * 128] for c in range(NB)]
                rr = row + r0
                pos = i * R + (rr % 8) * G + rr // 8
                logits = []
                for w in range(W):
                    off = r0 + (HALO - DIL * w) * 8
                    p = None
                    for c in range(NB):
                        t = qs[c] * kext[off:off + AG, c * 128:(c + 1) * 128]
                        p = t if p is None else p + t
                    p = p + jnp.where(lane % 2 == 0, pltpu.roll(p, 127, 1), pltpu.roll(p, 1, 1))
                    p = p + jnp.where(lane % 4 < 2, pltpu.roll(p, 126, 1), pltpu.roll(p, 2, 1))
                    if masked and r0 // 8 < DIL * w:
                        p = jnp.where(pos >= DIL * w, p, NEG)
                    logits.append(p)
                m = logits[0]
                for w in range(1, W):
                    m = jnp.maximum(m, logits[w])
                es = [jnp.exp(l - m) for l in logits]
                den = es[0]
                for w in range(1, W):
                    den = den + es[w]
                inv = 1.0 / den
                outs = []
                for c in range(NB):
                    acc = None
                    for w in range(W):
                        off = r0 + (HALO - DIL * w) * 8
                        t = es[w] * vext[off:off + AG, c * 128:(c + 1) * 128]
                        acc = t if acc is None else acc + t
                    outs.append(pltpu.bitcast((acc * inv).astype(BF16), jnp.uint32))
                outs = _butterfly(outs, AG // 2)
                for c in range(NB):
                    ob_s[r0:r0 + AG, c * 128:(c + 1) * 128] = pltpu.bitcast(outs[c], BF16)
                if chain:
                    q_s[pl.ds(qpad, 8), 0:128] = pltpu.bitcast(outs[NB - 1], F32)[0:8]

        def stage_wo(slot):
            att = jnp.dot(ob_s[...], wo_s[...], preferred_element_type=F32)
            h_s[slot] = xp_s[slot] + att

        def stage_ln2(slot):
            for r in range(R // AR):
                ln2_s[r * AR:(r + 1) * AR, :] = _ln(h_s[slot, r * AR:(r + 1) * AR, :]).astype(BF16)

        def stage_out(outp):
            for g in range(G):
                for c in range(NB):
                    xo_s[c, pl.ds(g, 8, stride=G), :] = outp[g * 8:(g + 1) * 8, c * 128:(c + 1) * 128]
            for c in range(NB):
                o_ref[:, c * 128:(c + 1) * 128] = xo_s[c].astype(BF16)

        def stage_ffn_out(slot):
            ln2 = ln2_s[...]
            acc = None
            for f in range(NFC):
                h1 = jnp.dot(ln2, w1_s[:, f * FC:(f + 1) * FC], preferred_element_type=F32)
                h1 = jnp.maximum(h1, 0.0).astype(BF16)
                t = jnp.dot(h1, w2_s[f * FC:(f + 1) * FC, :], preferred_element_type=F32)
                acc = t if acc is None else acc + t
            stage_out(h_s[slot] + acc)

        @pl.when(i == 0)
        def _():
            cp_p[0].start()
            kext[...] = jnp.zeros_like(kext)
            vext[...] = jnp.zeros_like(vext)
            stage_x(x0_ref, 0, lnp_s.at[0:R])
            stage_x(xn_ref, 1, lnp_s.at[R:2 * R])
            cp_p[1].start()
            cp_p[0].wait()
            cp_p[2].start()
            cp_wo.start()
            cp_w1(0).start()
            cp_w2(0).start()
            perm_w(0)
            cp_p[1].wait()
            for f in range(1, NF2):
                cp_w1(f).start()
                cp_w2(f).start()
            put_q(proj2(0))
            perm_w(1)
            cp_p[2].wait()
            put_kv(kext, proj2(1))
            perm_w(2)
            put_kv(vext, proj2(2))
            cp_wo.wait()

        @pl.when(i == 1)
        def _():
            put_q(stg_s[:, 0:D])
            put_kv(kext, stg_s[:, D:2 * D])
            put_kv(vext, stg_s[:, 2 * D:3 * D])

        @pl.when(i <= 1)
        def _():
            slot = i % 2
            stage_att(True, False)
            stage_x(xn_ref, 1 - slot, ln1_s)
            stage_wo(slot)

        @pl.when(jnp.logical_and(i > 1, i < NBLK))
        def _():
            slot = i % 2
            put_q(proj(0))
            put_kv(kext, proj(1))
            put_kv(vext, proj(2))
            stage_ln2(1 - slot)
            stage_ffn_out(1 - slot)
            stage_att(False, True)
            stage_x(xn_ref, 1 - slot, ln1_s)
            stage_wo(slot)

        @pl.when(jnp.logical_or(i == 1, i == NBLK))
        def _():
            slot = (i - 1) % 2
            stage_ln2(slot)
            acc_s[...] = h_s[slot]

            def body(f, carry):
                @pl.when(i == 1)
                def _():
                    cp_w1(f).wait()
                    cp_w2(f).wait()
                f0 = pl.multiple_of(f * FC2, 128)
                h1 = jnp.dot(ln2_s[...], w1_s[:, pl.ds(f0, FC2)], preferred_element_type=F32)
                h1 = jnp.maximum(h1, 0.0).astype(BF16)
                acc_s[...] += jnp.dot(h1, w2_s[pl.ds(f0, FC2), :], preferred_element_type=F32)
                return carry
            lax.fori_loop(0, NF2, body, 0)
            stage_out(acc_s[...])

    scratch = [
        pltpu.VMEM((D, 3 * D), BF16),
        pltpu.VMEM((D, 3 * D), BF16),
        pltpu.VMEM((D, D), BF16),
        pltpu.VMEM((D, DFF), BF16),
        pltpu.VMEM((DFF, D), BF16),
        pltpu.VMEM((NB, R, 128), F32),
        pltpu.VMEM((NB, R, 128), F32),
        pltpu.VMEM((2, R, D), F32),
        pltpu.VMEM((2, R, D), F32),
        pltpu.VMEM((R, D), F32),
        pltpu.VMEM((R + 8, D), F32),
        pltpu.VMEM(((G + HALO) * 8, D), F32),
        pltpu.VMEM(((G + HALO) * 8, D), F32),
        pltpu.VMEM((R, D), BF16),
        pltpu.VMEM((R, D), BF16),
        pltpu.VMEM((R, D), BF16),
        pltpu.VMEM((2 * R, D), BF16),
        pltpu.VMEM((R, 3 * D), F32),
        pltpu.SMEM((1,), jnp.int32),
        pltpu.SemaphoreType.DMA((4,)),
        pltpu.SemaphoreType.DMA((2, NF2)),
    ]
    return kernel, scratch, NBLK


def run(A_x, A_wqkv, A_wo, B_x, B_w1, B_w2, R=128, FC=1792, AR=32, PC=128, AG=16, FC2=896):
    kernel, scratch, NBLK = make_kernel(R, FC, AR, PC, AG, FC2)
    x = A_x.reshape(S, D)
    out = pl.pallas_call(
        kernel,
        grid=(NBLK + 1,),
        in_specs=[
            pl.BlockSpec((R, D), lambda i: (0, 0)),
            pl.BlockSpec((R, D), lambda i: (jnp.minimum(i + 1, NBLK - 1), 0)),
            pl.BlockSpec(memory_space=pl.ANY),
            pl.BlockSpec(memory_space=pl.ANY),
            pl.BlockSpec(memory_space=pl.ANY),
            pl.BlockSpec(memory_space=pl.ANY),
        ],
        out_specs=pl.BlockSpec((R, D), lambda i: (jnp.maximum(i - 1, 0), 0)),
        out_shape=jax.ShapeDtypeStruct((S, D), BF16),
        scratch_shapes=scratch,
        compiler_params=pltpu.CompilerParams(
            dimension_semantics=("arbitrary",),
            vmem_limit_bytes=100 * 1024 * 1024,
        ),
    )(x, x, A_wqkv, A_wo, B_w1, B_w2)
    return out.reshape(1, S, D)


@jax.jit
def pallas_sequential_preLN__sliding_local_dilated__dense_activation_relu__prompt_kernel(A_x, A_wqkv, A_wo, B_x, B_w1, B_w2):
    return run(A_x, A_wqkv, A_wo, B_x, B_w1, B_w2)
```
